```python
import jax
import jax.numpy as jnp

def _softmax(x, axis=-1):
    return jax.nn.softmax(x, axis=axis)

def _gelu(x):
    return jax.nn.gelu(x, approximate=True)

def _silu(x):
    return jax.nn.silu(x)

def _sigmoid(x):
    return jax.nn.sigmoid(x)

def _layernorm(x, axis=-1, eps=1e-05):
    m = jnp.mean(x, axis=axis, keepdims=True)
    v = jnp.var(x, axis=axis, keepdims=True)
    return (x - m) / jnp.sqrt(v + eps)

def _scatter_add(tgt, idx, src, axis=0):
    return tgt.at[idx].add(src)

def _segment_sum(src, seg, n):
    return jax.ops.segment_sum(src, seg, n)

class _Rng:

    def __init__(self, key):
        self._k = key

    def _next(self):
        self._k, sub = jax.random.split(self._k)
        return sub

    def normal(self, shape):
        return jax.random.normal(self._next(), shape, dtype=jnp.bfloat16)

    def randint(self, lo, hi, shape):
        return jax.random.randint(self._next(), shape, lo, hi, dtype=jnp.int32)

    def uniform(self, shape, lo=0.0, hi=1.0):
        return jax.random.uniform(self._next(), shape, jnp.bfloat16, lo, hi)

    def permutation(self, n):
        return jax.random.permutation(self._next(), n)
kernel_name = 'adaLN_cond__sliding_local_dilated__mixer_s_mlp__prompt'

def setup_inputs():
    _rng = _Rng(jax.random.key(int.from_bytes(__import__("os").urandom(4), "little")))
    _w = lambda a: (lambda t: t.astype(jnp.bfloat16) if jnp.issubdtype(t.dtype, jnp.floating) else t)(jnp.asarray(a))

    def _A_setup():
        B, S, D = (1, 2048, 1024)
        return {'x': _w((lambda *s: _rng.normal(s) * 0.05)(B, S, D)), 'wqkv': _w((lambda *s: _rng.normal(s) * 0.05)(D, 3 * D)), 'wo': _w((lambda *s: _rng.normal(s) * 0.05)(D, D))}
    _A_in = _A_setup()

    def _B_setup():
        B, S, D, F = (1, 2048, 1024, 3584)
        return {'x': _w((lambda *s: _rng.normal(s) * 0.05)(B, S, D)), 'w1': _w((lambda *s: _rng.normal(s) * 0.05)(D, D) * D ** (-0.5)), 'w2': _w((lambda *s: _rng.normal(s) * 0.05)(D, D) * D ** (-0.5)), 'w3': _w((lambda *s: _rng.normal(s) * 0.05)(D, F) * D ** (-0.5)), 'w4': _w((lambda *s: _rng.normal(s) * 0.05)(F, D) * F ** (-0.5))}
    _B_in = _B_setup()
    return {'A_x': _A_in['x'], 'A_wqkv': _A_in['wqkv'], 'A_wo': _A_in['wo'], 'B_x': _B_in['x'], 'B_w1': _B_in['w1'], 'B_w2': _B_in['w2'], 'B_w3': _B_in['w3'], 'B_w4': _B_in['w4'], 'c': _w((lambda *s: _rng.normal(s) * 0.05)(1, 1024)), 'w_mod': _w((lambda *s: _rng.normal(s) * 0.05)(1024, 6 * 1024) * 1024 ** (-0.5))}

def reference(A_x, A_wqkv, A_wo, B_x, B_w1, B_w2, B_w3, B_w4, c, w_mod):

    def _A_ref(x, wqkv, wo):
        B, S, D = x.shape
        H = 32
        Dh = D // H
        W, dil = (8, 2)
        qkv = (lambda x, *d: x.transpose(*d))((x @ wqkv).reshape(B, S, 3, H, Dh), 2, 0, 3, 1, 4)
        q, k, v = (qkv[0], qkv[1], qkv[2])
        scale = Dh ** (-0.5)
        pos = jnp.arange(S)
        off = jnp.arange(W) * dil
        idx = pos[:, None] - off[None, :]
        mask = idx >= 0
        idx_c = jnp.where(mask, idx, 0).reshape(-1)
        kg = k[:, :, idx_c, :].reshape(B, H, S, W, Dh)
        vg = v[:, :, idx_c, :].reshape(B, H, S, W, Dh)
        logits = jnp.einsum('bhsd,bhswd->bhsw', q, kg) * scale
        logits = jnp.where(mask[None, None, :, :], logits, -1000000000.0)
        attn = _softmax(logits, axis=-1)
        o = jnp.einsum('bhsw,bhswd->bhsd', attn, vg)
        return (lambda x, *d: x.transpose(*d))(o, 0, 2, 1, 3).reshape(B, S, D) @ wo

    def _B_ref(x, w1, w2, w3, w4):
        B, S, D = x.shape
        h = _gelu(_layernorm(x, axis=-1) @ w1)
        c = D // 4
        g0 = jnp.pad(h[:, :, 0 * c:1 * c], ((0, 0), (1, 0), (0, 0)))[:, :S, :]
        g1 = jnp.pad(h[:, :, 1 * c:2 * c], ((0, 0), (0, 1), (0, 0)))[:, 1:, :]
        g2 = jnp.pad(h[:, :, 2 * c:3 * c], ((0, 0), (2, 0), (0, 0)))[:, :S, :]
        g3 = jnp.pad(h[:, :, 3 * c:], ((0, 0), (0, 2), (0, 0)))[:, 2:, :]
        hs = jnp.concatenate([g0, g1, g2, g3], axis=-1) @ w2
        x1 = x + hs
        h2 = _gelu(_layernorm(x1, axis=-1) @ w3) @ w4
        return x1 + h2
    x = A_x
    mod = (_silu(c) @ w_mod).reshape(c.shape[0], 6, 1, -1)
    sa, ca, ga, sb, cb, gb = (mod[:, 0].copy(), mod[:, 1].copy(), mod[:, 2].copy(), mod[:, 3].copy(), mod[:, 4].copy(), mod[:, 5].copy())
    h = _layernorm(x, axis=-1) * (1 + ca) + sa
    x = x + ga * _A_ref(h, A_wqkv, A_wo)
    h = _layernorm(x, axis=-1) * (1 + cb) + sb
    x = x + gb * _B_ref(h, B_w1, B_w2, B_w3, B_w4)
    return x
```

```python
import jax
import jax.numpy as jnp
import jax.experimental.pallas as pl
import jax.experimental.pallas.tpu as pltpu

S, D, F = 2048, 1024, 3584
TM = 128
N = S // TM
FC = 512
W, DIL, DH = 8, 2, 32
f32, bf16 = jnp.float32, jnp.bfloat16


def _ln(x):
    m = jnp.mean(x, axis=-1, keepdims=True)
    d = x - m
    v = jnp.mean(d * d, axis=-1, keepdims=True)
    return d * jax.lax.rsqrt(v + 1e-5)


def _gelu(x):
    u = x * (0.7978845608028654 + 0.7978845608028654 * 0.044715 * (x * x))
    h = 0.5 * x
    return h + h * jnp.tanh(u)


def _dot(a, b):
    return jnp.dot(a, b, preferred_element_type=f32)


def _kernel(x0_ref, x1_ref, c_ref, wm_h, wqkv_h, wo_h, w1_h, w2_h, w3_h, w4_h, o_ref,
            wm, wqkv, wo, w1, w2, w3, w4, mod, kb, vb, hb, xb, bb, sem):
    i = pl.program_id(0)

    def cp(j):
        if j < 6:
            s = (slice(None), slice(j * D, (j + 1) * D))
            return pltpu.make_async_copy(wm_h.at[s], wm.at[s], sem.at[j])
        if j < 9:
            s = (slice(None), slice((j - 6) * D, (j - 5) * D))
            return pltpu.make_async_copy(wqkv_h.at[s], wqkv.at[s], sem.at[j])
        a, b = ((wo_h, wo), (w1_h, w1), (w2_h, w2), (w3_h, w3), (w4_h, w4))[j - 9]
        return pltpu.make_async_copy(a, b, sem.at[j])

    def domod(j):
        cp(j).wait()
        c = jnp.broadcast_to(c_ref[...].astype(f32), (16, D))
        sc = (c * jax.nn.sigmoid(c)).astype(bf16)
        r = _dot(sc, wm[:, j * D:(j + 1) * D])[:8]
        mod[j] = r + 1.0 if j in (1, 4) else r

    def m(j):
        return mod[j][0:1, :]

    def p1(x_ref, t, first):
        r0 = t * TM if first else pl.multiple_of(t * TM, TM)
        x = x_ref[...].astype(f32)
        h = (_ln(x) * m(1) + m(0)).astype(bf16)
        if first:
            kb[0:16, :] = jnp.zeros((16, D), f32)
            vb[0:16, :] = jnp.zeros((16, D), f32)
            cp(7).wait()
        else:
            kb[0:16, :] = kb[TM:TM + 16, :]
            vb[0:16, :] = vb[TM:TM + 16, :]
        kb[16:, :] = _dot(h, wqkv[:, D:2 * D])
        if first:
            cp(8).wait()
        vb[16:, :] = _dot(h, wqkv[:, 2 * D:])
        if first:
            cp(6).wait()
        q = _dot(h, wqkv[:, :D]) * (DH ** -0.5)
        bd = (jax.lax.broadcasted_iota(jnp.int32, (128, 128), 0) // DH ==
              jax.lax.broadcasted_iota(jnp.int32, (128, 128), 1) // DH).astype(bf16)
        outs = []
        for cch in range(D // 128):
            cs = slice(cch * 128, (cch + 1) * 128)
            qc = q[:, cs]
            lg = []
            for w in range(W):
                o = 16 - DIL * w
                l = _dot((qc * kb[o:o + TM, cs]).astype(bf16), bd)
                if first and w:
                    row = jax.lax.broadcasted_iota(jnp.int32, (TM, 128), 0)
                    l = jnp.where(row >= DIL * w, l, -1e9)
                lg.append(l)
            mx = lg[0]
            for l in lg[1:]:
                mx = jnp.maximum(mx, l)
            den = acc = None
            for w in range(W):
                o = 16 - DIL * w
                e = jnp.exp(lg[w] - mx)
                pv = e * vb[o:o + TM, cs]
                den = e if den is None else den + e
                acc = pv if acc is None else acc + pv
            outs.append((acc * pl.reciprocal(den, approx=True)).astype(bf16))
        a = jnp.concatenate(outs, axis=1)
        if first:
            cp(9).wait()
            domod(2)
            domod(3)
            domod(4)
        x = x + m(2) * _dot(a, wo[...])
        xb[pl.ds(r0, TM), :] = x
        b = _ln(x) * m(4) + m(3)
        bb[pl.ds(r0, TM), :] = b
        if first:
            cp(10).wait()
        hb[pl.ds(r0 + 8, TM), :] = _gelu(_dot(_ln(b).astype(bf16), w1[...]))

    def p2(t):
        r0 = pl.multiple_of(t * TM, TM)
        c = D // 4
        parts = []
        for g, sh in enumerate((-1, 1, -2, 2)):
            win = hb[pl.ds(r0, TM + 16), g * c:(g + 1) * c]
            parts.append(win[8 + sh:8 + sh + TM].astype(bf16))
        x1 = bb[pl.ds(r0, TM), :] + _dot(jnp.concatenate(parts, axis=1), w2[...])
        n = _ln(x1).astype(bf16)
        acc = x1
        for f in range(F // FC):
            fs = slice(f * FC, (f + 1) * FC)
            acc = acc + _dot(_gelu(_dot(n, w3[:, fs])).astype(bf16), w4[fs, :])
        o_ref[...] = (xb[pl.ds(r0, TM), :] + m(5) * acc).astype(o_ref.dtype)

    @pl.when(i == 0)
    def _():
        for j in (0, 1, 7, 8, 6, 9, 2, 3, 4, 10, 11, 12, 5, 13):
            cp(j).start()
        hb[0:8, :] = jnp.zeros((8, D), f32)
        hb[S + 8:, :] = jnp.zeros((8, D), f32)
        domod(0)
        domod(1)
        p1(x0_ref, 0, True)
        for j in (11, 12, 13):
            cp(j).wait()
        domod(5)

    @pl.when(i < N - 1)
    def _():
        p1(x1_ref, i + 1, False)
        p2(i)

    @pl.when(i == N - 1)
    def _():
        p2(i)


@jax.jit
def pallas_adaLN_cond__sliding_local_dilated__mixer_s_mlp__prompt_kernel(
        A_x, A_wqkv, A_wo, B_x, B_w1, B_w2, B_w3, B_w4, c, w_mod):
    x = A_x.reshape(S, D)
    anyspec = pl.BlockSpec(memory_space=pl.ANY)
    V = pltpu.VMEM
    out = pl.pallas_call(
        _kernel,
        grid=(N,),
        in_specs=[pl.BlockSpec((TM, D), lambda i: (0, 0)),
                  pl.BlockSpec((TM, D), lambda i: (jnp.minimum(i + 1, N - 1), 0)),
                  pl.BlockSpec((1, D), lambda i: (0, 0))] + [anyspec] * 7,
        out_specs=pl.BlockSpec((TM, D), lambda i: (i, 0)),
        out_shape=jax.ShapeDtypeStruct((S, D), bf16),
        scratch_shapes=[V((D, 6 * D), bf16), V((D, 3 * D), bf16), V((D, D), bf16),
                        V((D, D), bf16), V((D, D), bf16), V((D, F), bf16), V((F, D), bf16),
                        V((6, 8, D), f32), V((TM + 16, D), f32), V((TM + 16, D), f32),
                        V((S + 16, D), f32), V((S, D), f32), V((S, D), f32),
                        pltpu.SemaphoreType.DMA((14,))],
        compiler_params=pltpu.CompilerParams(
            dimension_semantics=("arbitrary",), vmem_limit_bytes=110 * 1024 * 1024),
    )(x, x, c, w_mod, A_wqkv, A_wo, B_w1, B_w2, B_w3, B_w4)
    return out.reshape(1, S, D)
```
